```python
import jax
import jax.numpy as jnp

def _softmax(x, axis=-1):
    return jax.nn.softmax(x, axis=axis)

def _gelu(x):
    return jax.nn.gelu(x, approximate=True)

def _silu(x):
    return jax.nn.silu(x)

def _sigmoid(x):
    return jax.nn.sigmoid(x)

def _layernorm(x, axis=-1, eps=1e-05):
    m = jnp.mean(x, axis=axis, keepdims=True)
    v = jnp.var(x, axis=axis, keepdims=True)
    return (x - m) / jnp.sqrt(v + eps)

def _scatter_add(tgt, idx, src, axis=0):
    return tgt.at[idx].add(src)

def _segment_sum(src, seg, n):
    return jax.ops.segment_sum(src, seg, n)

class _Rng:

    def __init__(self, key):
        self._k = key

    def _next(self):
        self._k, sub = jax.random.split(self._k)
        return sub

    def normal(self, shape):
        return jax.random.normal(self._next(), shape, dtype=jnp.bfloat16)

    def randint(self, lo, hi, shape):
        return jax.random.randint(self._next(), shape, lo, hi, dtype=jnp.int32)

    def uniform(self, shape, lo=0.0, hi=1.0):
        return jax.random.uniform(self._next(), shape, jnp.bfloat16, lo, hi)

    def permutation(self, n):
        return jax.random.permutation(self._next(), n)
kernel_name = 'adaLN_cond__sliding_block_cached__glu_gated_bilinear__decode'

def setup_inputs():
    _rng = _Rng(jax.random.key(int.from_bytes(__import__("os").urandom(4), "little")))
    _w = lambda a: (lambda t: t.astype(jnp.bfloat16) if jnp.issubdtype(t.dtype, jnp.floating) else t)(jnp.asarray(a))

    def _A_setup():
        B, Sq, D = (1, 1, 640)
        Hq, Hkv, Sk, Dh = (32, 32, 32768, 192)
        assert Hq % Hkv == 0, (Hq, Hkv)
        return {'x': _w((lambda *s: _rng.normal(s) * 0.05)(B, Sq, D)), 'k_cache': _w((lambda *s: _rng.normal(s) * 0.05)(B, Hkv, Sk, Dh)), 'v_cache': _w((lambda *s: _rng.normal(s) * 0.05)(B, Hkv, Sk, Dh)), 'wq': _w((lambda *s: _rng.normal(s) * 0.05)(D, Hq * Dh) * D ** (-0.5)), 'wo': _w((lambda *s: _rng.normal(s) * 0.05)(Hq * Dh, D) * (Hq * Dh) ** (-0.5))}
    _A_in = _A_setup()

    def _B_setup():
        B, S, D, F = (1, 1, 640, 1536)
        return {'x': _w((lambda *s: _rng.normal(s) * 0.05)(B, S, D)), 'w_gate': _w((lambda *s: _rng.normal(s) * 0.05)(D, F) * D ** (-0.5)), 'w_up': _w((lambda *s: _rng.normal(s) * 0.05)(D, F) * D ** (-0.5)), 'w_down': _w((lambda *s: _rng.normal(s) * 0.05)(F, D) * F ** (-0.5))}
    _B_in = _B_setup()
    return {'A_x': _A_in['x'], 'A_k_cache': _A_in['k_cache'], 'A_v_cache': _A_in['v_cache'], 'A_wq': _A_in['wq'], 'A_wo': _A_in['wo'], 'B_x': _B_in['x'], 'B_w_gate': _B_in['w_gate'], 'B_w_up': _B_in['w_up'], 'B_w_down': _B_in['w_down'], 'c': _w((lambda *s: _rng.normal(s) * 0.05)(1, 640)), 'w_mod': _w((lambda *s: _rng.normal(s) * 0.05)(640, 6 * 640) * 640 ** (-0.5))}

def reference(A_x, A_k_cache, A_v_cache, A_wq, A_wo, B_x, B_w_gate, B_w_up, B_w_down, c, w_mod):

    def _A_ref(x, k_cache, v_cache, wq, wo):
        B, Sq, D = x.shape
        Hq, Dh = (32, 192)
        Hkv, Sk = (k_cache.shape[1], k_cache.shape[2])
        W = min(4096, max(256, Sk // 4))
        rep = Hq // Hkv
        q = (lambda x, *d: x.transpose(*d))((x @ wq).reshape(B, Sq, Hq, Dh), 0, 2, 1, 3)
        k = jnp.repeat(k_cache[:, :, Sk - W:, :], rep, axis=1)
        v = jnp.repeat(v_cache[:, :, Sk - W:, :], rep, axis=1)
        scores = jnp.einsum('bhqd,bhkd->bhqk', q, k) * Dh ** (-0.5)
        p = _softmax(scores, axis=-1)
        o = jnp.einsum('bhqk,bhkd->bhqd', p, v)
        return (lambda x, *d: x.transpose(*d))(o, 0, 2, 1, 3).reshape(B, Sq, Hq * Dh) @ wo

    def _B_ref(x, w_gate, w_up, w_down):
        g = jnp.einsum('bsd,df->bsf', x, w_gate)
        u = jnp.einsum('bsd,df->bsf', x, w_up)
        h = g * u
        return jnp.einsum('bsf,fd->bsd', h, w_down)
    x = A_x
    mod = (_silu(c) @ w_mod).reshape(c.shape[0], 6, 1, -1)
    sa, ca, ga, sb, cb, gb = (mod[:, 0].copy(), mod[:, 1].copy(), mod[:, 2].copy(), mod[:, 3].copy(), mod[:, 4].copy(), mod[:, 5].copy())
    h = _layernorm(x, axis=-1) * (1 + ca) + sa
    x = x + ga * _A_ref(h, A_k_cache, A_v_cache, A_wq, A_wo)
    h = _layernorm(x, axis=-1) * (1 + cb) + sb
    x = x + gb * _B_ref(h, B_w_gate, B_w_up, B_w_down)
    return x
```

```python
import functools
import jax
import jax.numpy as jnp
import numpy as np
from jax import lax
from jax.experimental import pallas as pl
from jax.experimental.pallas import tpu as pltpu

D = 640
HQ, DH = 32, 192
SK, W = 32768, 4096
F = 1536
PR = 2 * DH
NP = HQ // 2
EPS = 1e-5
LOG2E = 1.4426950408889634
SCALE = DH ** -0.5


def _mm(a, b):
    return jnp.dot(a, b, preferred_element_type=jnp.float32)


def _mm_nt(a, b):
    return lax.dot_general(a, b, (((1,), (1,)), ((), ())), preferred_element_type=jnp.float32)


def _layernorm(x):
    m = jnp.mean(x, axis=-1, keepdims=True)
    d = x - m
    v = jnp.mean(d * d, axis=-1, keepdims=True)
    return d * lax.rsqrt(v + EPS)


def _make(nslot=2, wd_chunks=6, wq_chunks=5):
    WDR = F // wd_chunks
    WQR = D // wq_chunks

    def kernel(x_hbm, c_hbm, wmod_hbm, wq_hbm, kt_hbm, vt_hbm, wo_hbm, wg_hbm, wu_hbm, wd_hbm,
               o_ref,
               x_v, c_v, wmod_v, wq_v, k_v, v_v, wo_v, wg_v, wu_v, wd_v, q_v,
               sem_s, sem_q, sem_k, sem_v, sem_o, sem_d):
        def k_copy(p, slot):
            return pltpu.make_async_copy(
                kt_hbm.at[pl.ds(pl.multiple_of(p * PR, PR), PR), pl.ds(SK - W, W)], k_v.at[slot], sem_k.at[slot])

        def v_copy(p, slot):
            return pltpu.make_async_copy(
                vt_hbm.at[pl.ds(pl.multiple_of(p * PR, PR), PR), pl.ds(SK - W, W)], v_v.at[slot], sem_v.at[slot])

        def o_copy(p, slot):
            return pltpu.make_async_copy(
                wo_hbm.at[pl.ds(pl.multiple_of(p * PR, PR), PR), :], wo_v.at[slot], sem_o.at[slot])

        c_cp = pltpu.make_async_copy(c_hbm, c_v, sem_s.at[0])
        x_cp = pltpu.make_async_copy(x_hbm, x_v, sem_s.at[1])
        mod_cp = pltpu.make_async_copy(wmod_hbm, wmod_v, sem_s.at[2])
        wg_cp = pltpu.make_async_copy(wg_hbm, wg_v, sem_s.at[3])
        wu_cp = pltpu.make_async_copy(wu_hbm, wu_v, sem_s.at[4])
        wq_cp = [pltpu.make_async_copy(wq_hbm.at[pl.ds(i * WQR, WQR), :], wq_v.at[pl.ds(i * WQR, WQR), :], sem_q.at[i])
                 for i in range(wq_chunks)]
        wd_cp = [pltpu.make_async_copy(wd_hbm.at[pl.ds(i * WDR, WDR), :], wd_v.at[pl.ds(i * WDR, WDR), :], sem_d.at[i])
                 for i in range(wd_chunks)]

        mod_cp.start()
        c_cp.start()
        x_cp.start()
        for cp in wq_cp:
            cp.start()
        for s in range(nslot):
            k_copy(s, s).start()
            v_copy(s, s).start()
            o_copy(s, s).start()

        c_cp.wait()
        x_cp.wait()
        cf = c_v[...].astype(jnp.float32)
        sc = cf * jax.nn.sigmoid(cf)
        sc8 = jnp.broadcast_to(sc, (8, D)).astype(jnp.bfloat16)
        xf = x_v[0].astype(jnp.float32)
        xf8 = jnp.broadcast_to(xf, (8, D))
        ln1 = _layernorm(xf8)
        mod_cp.wait()
        mod = _mm(sc8, wmod_v[...])
        mod = mod.astype(jnp.bfloat16).astype(jnp.float32)
        sa, ca, ga = mod[:, 0:D], mod[:, D:2 * D], mod[:, 2 * D:3 * D]
        sb, cb, gb = mod[:, 3 * D:4 * D], mod[:, 4 * D:5 * D], mod[:, 5 * D:6 * D]
        h1 = (ln1 * (1.0 + ca) + sa).astype(jnp.bfloat16)

        q = jnp.zeros((8, HQ * DH), jnp.float32)
        for i, cp in enumerate(wq_cp):
            cp.wait()
            q = q + _mm(h1[:, i * WQR:(i + 1) * WQR], wq_v[i * WQR:(i + 1) * WQR, :])
        sub = lax.broadcasted_iota(jnp.int32, (8, HQ * DH), 0)
        lane = lax.broadcasted_iota(jnp.int32, (8, HQ * DH), 1)
        q = jnp.where(((lane // DH) % 2) == sub, q, 0.0)
        for p in range(NP):
            q_v[p] = q[:, p * PR:(p + 1) * PR].astype(jnp.bfloat16)

        sub_p = lax.broadcasted_iota(jnp.int32, (8, PR), 0)
        lane_p = lax.broadcasted_iota(jnp.int32, (8, PR), 1)
        pair_mask = (lane_p >= DH).astype(jnp.int32) == sub_p

        def body(p, acc):
            slot = p % nslot
            k_copy(p, slot).wait()
            s = _mm(q_v[p], k_v[slot])

            @pl.when(p + nslot < NP)
            def _():
                k_copy(p + nslot, slot).start()

            @pl.when(p + nslot == NP)
            def _():
                wg_cp.start()

            m = jnp.max(s, axis=-1, keepdims=True)
            e = jnp.exp2((s - m) * (SCALE * LOG2E))
            l = jnp.sum(e, axis=-1, keepdims=True)
            eb = e.astype(jnp.bfloat16)
            v_copy(p, slot).wait()
            o = _mm_nt(eb, v_v[slot])

            @pl.when(p + nslot < NP)
            def _():
                v_copy(p + nslot, slot).start()

            @pl.when(p + nslot == NP)
            def _():
                wu_cp.start()

            o = jnp.where(pair_mask, o * (1.0 / l), 0.0).astype(jnp.bfloat16)
            o_copy(p, slot).wait()
            acc = acc + _mm(o, wo_v[slot])

            @pl.when(p + nslot < NP)
            def _():
                o_copy(p + nslot, slot).start()

            @pl.when(p + nslot == NP)
            def _():
                for cp in wd_cp:
                    cp.start()

            return acc

        acc = lax.fori_loop(0, NP, body, jnp.zeros((8, D), jnp.float32))
        attn = jnp.sum(acc, axis=0, keepdims=True)
        x1 = xf8 + ga * attn
        h2 = (_layernorm(x1) * (1.0 + cb) + sb).astype(jnp.bfloat16)

        wg_cp.wait()
        g = _mm(h2, wg_v[...])
        wu_cp.wait()
        u = _mm(h2, wu_v[...])
        hh = (g * u).astype(jnp.bfloat16)
        y = jnp.zeros((8, D), jnp.float32)
        for i, cp in enumerate(wd_cp):
            cp.wait()
            y = y + _mm(hh[:, i * WDR:(i + 1) * WDR], wd_v[i * WDR:(i + 1) * WDR, :])
        out = x1 + gb * y
        o_ref[0] = out[0:1, :].astype(jnp.bfloat16)

    def fn(A_x, A_k_cache, A_v_cache, A_wq, A_wo, B_x, B_w_gate, B_w_up, B_w_down, c, w_mod):
        del B_x
        kt = A_k_cache.transpose(0, 1, 3, 2).reshape(HQ * DH, SK)
        vt = A_v_cache.transpose(0, 1, 3, 2).reshape(HQ * DH, SK)
        hbm = pl.BlockSpec(memory_space=pl.ANY)
        return pl.pallas_call(
            kernel,
            in_specs=[hbm] * 10,
            out_specs=pl.BlockSpec(memory_space=pltpu.VMEM),
            out_shape=jax.ShapeDtypeStruct((1, 1, D), jnp.bfloat16),
            scratch_shapes=[
                pltpu.VMEM((1, 1, D), jnp.bfloat16),
                pltpu.VMEM((1, D), jnp.bfloat16),
                pltpu.VMEM((D, 6 * D), jnp.bfloat16),
                pltpu.VMEM((D, HQ * DH), jnp.bfloat16),
                pltpu.VMEM((nslot, PR, W), jnp.bfloat16),
                pltpu.VMEM((nslot, PR, W), jnp.bfloat16),
                pltpu.VMEM((nslot, PR, D), jnp.bfloat16),
                pltpu.VMEM((D, F), jnp.bfloat16),
                pltpu.VMEM((D, F), jnp.bfloat16),
                pltpu.VMEM((F, D), jnp.bfloat16),
                pltpu.VMEM((NP, 8, PR), jnp.bfloat16),
                pltpu.SemaphoreType.DMA((5,)),
                pltpu.SemaphoreType.DMA((wq_chunks,)),
                pltpu.SemaphoreType.DMA((nslot,)),
                pltpu.SemaphoreType.DMA((nslot,)),
                pltpu.SemaphoreType.DMA((nslot,)),
                pltpu.SemaphoreType.DMA((wd_chunks,)),
            ],
            compiler_params=pltpu.CompilerParams(vmem_limit_bytes=100 * 1024 * 1024),
        )(A_x, c, w_mod, A_wq, kt, vt, A_wo, B_w_gate, B_w_up, B_w_down)

    return fn


@jax.jit
def pallas_adaLN_cond__sliding_block_cached__glu_gated_bilinear__decode_kernel(
    A_x, A_k_cache, A_v_cache, A_wq, A_wo, B_x, B_w_gate, B_w_up, B_w_down, c, w_mod,
):
    return _make()(A_x, A_k_cache, A_v_cache, A_wq, A_wo, B_x, B_w_gate, B_w_up, B_w_down, c, w_mod)
```

```python
import contextlib
import jax
import jax.numpy as jnp
from jax import lax
from jax.experimental import pallas as pl
from jax.experimental.pallas import tpu as pltpu

D = 640
HQ, DH = 32, 192
SK, W = 32768, 4096
F = 1536
PR = 2 * DH
NP = HQ // 2
EPS = 1e-5
LOG2E = 1.4426950408889634
SCALE = DH ** -0.5


def _mm(a, b):
    return jnp.dot(a, b, preferred_element_type=jnp.float32)


def _mm_nt(a, b):
    return lax.dot_general(a, b, (((1,), (1,)), ((), ())), preferred_element_type=jnp.float32)


def _layernorm(x):
    m = jnp.mean(x, axis=-1, keepdims=True)
    d = x - m
    v = jnp.mean(d * d, axis=-1, keepdims=True)
    return d * lax.rsqrt(v + EPS)


def _make(GC=512, RP=128, LA=6, mod_cols=1920, wq_cols=2048, wd_chunks=6, wd_rows=32, checks=False,
         wq_pre=20, n_pre=3, up_tail=True, v_per=2, up_slots=5, wd_per=2, tail_gap=0, scopes=False,
         up_chunks=1, wo_rows=24, flags=None):
    NG = W // GC
    NJ = GC // 128
    NPART = PR // RP
    WDR = F // wd_chunks
    WO_N = PR // NG // wo_rows
    assert LA < NG and n_pre <= LA
    assert WDR % (2 * wd_rows) == 0
    lg = NG.bit_length() - 1
    assert 1 << lg == NG
    v_slots = NG // v_per
    up_a = v_slots
    up_n = up_slots if up_tail else 0
    assert (D // 8) % up_slots == 0
    up_per = D // 8 // up_slots
    wd_a = up_a + up_n + tail_gap
    wd_slots = wd_chunks // wd_per
    assert wd_a + wd_slots <= LA + NG, (wd_a, wd_slots, LA, NG)
    assert up_slots % up_chunks == 0 or not up_tail
    scope = jax.named_scope if scopes else (lambda name: contextlib.nullcontext())

    def kernel(x_hbm, c_hbm, wmod_hbm, wq_hbm, kt_hbm, vt_hbm, wo_hbm, wg_hbm, wu_hbm, wd_hbm,
               o_ref,
               x_v, c_v, wmod_v, wq_v, kv_v, wo_v, wg_v, wu_v, wd_v, s_v,
               sem_s, sem_k, sem_v, sem_o, sem_d, sem_u):
        k_v, v_v = kv_v.at[0], kv_v.at[1]

        def kv_dma(src, dst, sem, u, g, j, r0, nr, pr):
            r = pl.multiple_of(u * PR + r0, 8)
            cc = pl.multiple_of(SK - W + g * GC + j * 128, 128)
            slot = (u & 1) * NG + g
            pltpu.make_async_copy(src.at[pl.ds(r, nr), pl.ds(cc, 128)],
                                  dst.at[slot, pl.ds(r0, nr), pl.ds(j * 128, 128)],
                                  sem.at[slot]).start(priority=pr)

        def rows_dma(src, dst, sem, r, nr, pr, c0=0, nc=None):
            nc = src.shape[1] if nc is None else nc
            r = pl.multiple_of(r, 8)
            pltpu.make_async_copy(src.at[pl.ds(r, nr), pl.ds(c0, nc)], dst.at[pl.ds(r, nr), pl.ds(c0, nc)],
                                  sem).start(priority=pr)

        def issue_intra(src, dst, sem, u, g):
            for j in range(NJ):
                kv_dma(src, dst, sem, u, g, j, 0, DH, 0)
                kv_dma(src, dst, sem, u, g, j, DH, DH, 1)

        def issue_main(t, with_g):
            u = lax.shift_right_logical(t, lg)
            g = t & (NG - 1)
            for j in range(NJ):
                for part in range(NPART):
                    kv_dma(kt_hbm, k_v, sem_k, u + 1, g, j, part * RP, RP, 0)
                    kv_dma(vt_hbm, v_v, sem_v, u, g, j, part * RP, RP, 1)
            r = (u + 1) * PR + g * (WO_N * wo_rows)
            so = sem_o.at[(u + 1) & 3]
            for i in range(WO_N):
                rows_dma(wo_hbm, wo_v, so, r + i * wo_rows, wo_rows, i % 2)

            def gate():
                if up_tail:
                    rows_dma(wg_hbm, wg_v, sem_s.at[4], t * 8, 8, 0, 0, F // 2)
                    rows_dma(wg_hbm, wg_v, sem_s.at[4], t * 8, 8, 1, F // 2, F // 2)
                else:
                    rows_dma(wg_hbm, wg_v, sem_s.at[4], t * 8, 8, 0)
                    rows_dma(wu_hbm, wu_v, sem_u.at[0], t * 8, 8, 1)
            if with_g == "dyn":
                pl.when(t < D // 8)(gate)
            elif with_g:
                gate()

        def issue_tail(i, lo, hi):
            if lo < v_slots:
                @pl.when(i < v_slots)
                def _():
                    for k in range(v_per):
                        issue_intra(vt_hbm, v_v, sem_v, NP - 1, i * v_per + k)
            if up_n and lo < up_a + up_n and hi > up_a:
                @pl.when(jnp.logical_and(i >= up_a, i < up_a + up_n))
                def _():
                    su = sem_u.at[(i - up_a) // (up_slots // up_chunks)] if up_chunks > 1 else sem_u.at[0]
                    for k in range(up_per):
                        rows_dma(wu_hbm, wu_v, su, ((i - up_a) * up_per + k) * 8, 8, k % 2)
            if lo < wd_a + wd_slots and hi > wd_a:
                @pl.when(jnp.logical_and(i >= wd_a, i < wd_a + wd_slots))
                def _():
                    for k in range(wd_per):
                        ch = (i - wd_a) * wd_per + k
                        for n in range(WDR // wd_rows):
                            rows_dma(wd_hbm, wd_v, sem_d.at[ch], ch * WDR + n * wd_rows, wd_rows, n % 2)

        def issue_halves(src, dst, sem, cols, lo, hi):
            R, C = src.shape

            def body(i, _):
                for j in range(C // cols):
                    for half in range(2):
                        rows_dma(src, dst, sem, half * (R // 2) + i * 8, 8, half, j * cols, cols)
            if hi > lo:
                lax.fori_loop(lo, hi, body, None)

        def wait_all(dst, sem):
            pltpu.make_async_copy(dst, dst, sem).wait()

        c_cp = pltpu.make_async_copy(c_hbm, c_v, sem_s.at[0])
        x_cp = pltpu.make_async_copy(x_hbm, x_v, sem_s.at[1])

        with scope("issue_mod"):
            issue_halves(wmod_hbm, wmod_v, sem_s.at[2], mod_cols, 0, 2)
            c_cp.start()
            x_cp.start()
            issue_halves(wmod_hbm, wmod_v, sem_s.at[2], mod_cols, 2, D // 16)
        with scope("issue_wq_a"):
            issue_halves(wq_hbm, wq_v, sem_s.at[3], wq_cols, 0, wq_pre)

        with scope("mod"):
            c_cp.wait()
            x_cp.wait()
            cf = c_v[...].astype(jnp.float32)
            sc = cf * jax.nn.sigmoid(cf)
            sc8 = jnp.broadcast_to(sc, (8, D)).astype(jnp.bfloat16)
            xf8 = jnp.broadcast_to(x_v[0].astype(jnp.float32), (8, D))
            ln1 = _layernorm(xf8)
            wait_all(wmod_v, sem_s.at[2])
            mod = _mm(sc8, wmod_v[...])
            mod = mod.astype(jnp.bfloat16).astype(jnp.float32)
            sa, ca, ga = mod[:, 0:D], mod[:, D:2 * D], mod[:, 2 * D:3 * D]
            sb, cb, gb = mod[:, 3 * D:4 * D], mod[:, 4 * D:5 * D], mod[:, 5 * D:6 * D]
            h1 = (ln1 * (1.0 + ca) + sa).astype(jnp.bfloat16)

        with scope("issue_wq_b"):
            issue_halves(wq_hbm, wq_v, sem_s.at[3], wq_cols, wq_pre, D // 16)
        with scope("issue_k0"):
            lax.fori_loop(0, NG, lambda g, _: issue_intra(kt_hbm, k_v, sem_k, 0, g), None)
            for i in range(4):
                rows_dma(wo_hbm, wo_v, sem_o.at[0], i * (PR // 4), PR // 4, i % 2)
        with scope("issue_pre"):
            if n_pre:
                lax.fori_loop(0, n_pre, lambda t, _: issue_main(t, True), None)
        with scope("wait_wq"):
            wait_all(wq_v, sem_s.at[3])

        sub_p = lax.broadcasted_iota(jnp.int32, (8, PR), 0)
        lane_p = lax.broadcasted_iota(jnp.int32, (8, PR), 1)
        pair_mask = (lane_p >= DH).astype(jnp.int32) == sub_p

        def q_block(u):
            q = _mm(h1, wq_v[:, pl.ds(pl.multiple_of(u * PR, 128), PR)])
            return jnp.where(pair_mask, q, 0.0).astype(jnp.bfloat16)

        def scores(qb, par, g, m_run):
            s = _mm(qb, k_v[par * NG + g])
            s_v[par, g] = s
            for j in range(NJ):
                m_run = jnp.maximum(m_run, s[:, j * 128:(j + 1) * 128])
            return m_run

        def probs(par, g, m, l_run):
            e = jnp.exp2((s_v[par, g] - m) * (SCALE * LOG2E))
            for j in range(NJ):
                l_run = l_run + e[:, j * 128:(j + 1) * 128]
            return e.astype(jnp.bfloat16), l_run

        def finish_pair(u, o, l_run, acc):
            l = jnp.sum(l_run, axis=-1, keepdims=True)
            ob = jnp.where(pair_mask, o * (1.0 / l), 0.0).astype(jnp.bfloat16)
            r = pl.multiple_of(u * PR, PR)
            wait_all(wo_v.at[pl.ds(r, PR), :], sem_o.at[u & 3])
            return acc + _mm(ob, wo_v[pl.ds(r, PR), :])

        neg = jnp.full((8, 128), -jnp.inf, jnp.float32)
        zero_o = jnp.zeros((8, PR), jnp.float32)
        zero_l = jnp.zeros((8, 128), jnp.float32)

        qb0 = q_block(0)

        def k0_step(g, m_run):
            wait_all(k_v.at[g], sem_k.at[g])
            if n_pre < LA:
                @pl.when(g < LA - n_pre)
                def _():
                    issue_main(n_pre + g, True)
            return scores(qb0, 0, g, m_run)

        with scope("k0_loop"):
            m = jnp.max(lax.fori_loop(0, NG, k0_step, neg), axis=-1, keepdims=True)

        def pair_body(u, carry, last):
            m, acc = carry
            qb = q_block(u + 1)
            pv = u & 1

            def step(g, c2):
                m_run, o, l_run = c2
                t = u * NG + g
                sv, sk = pv * NG + g, (1 - pv) * NG + g
                wait_all(v_v.at[sv], sem_v.at[sv])
                wait_all(k_v.at[sk], sem_k.at[sk])
                if last:
                    @pl.when(g + LA < NG)
                    def _():
                        issue_main(t + LA, False)

                    @pl.when(g + LA >= NG)
                    def _():
                        issue_tail(g + LA - NG, 0, LA)
                else:
                    issue_main(t + LA, "dyn")
                eb, l_run = probs(pv, g, m, l_run)
                o = o + _mm_nt(eb, v_v[sv])
                m_run = scores(qb, 1 - pv, g, m_run)
                return m_run, o, l_run

            m_run, o, l_run = lax.fori_loop(0, NG, step, (neg, zero_o, zero_l))
            m_new = jnp.max(m_run, axis=-1, keepdims=True)
            return m_new, finish_pair(u, o, l_run, acc)

        with scope("main_loop"):
            carry = lax.fori_loop(0, NP - 2, lambda u, c_: pair_body(u, c_, False),
                                  (m, jnp.zeros((8, D), jnp.float32)))
        with scope("last_main"):
            m, acc = pair_body(NP - 2, carry, True)

        def v_step(g, c2):
            o, l_run = c2
            sv = ((NP - 1) & 1) * NG + g
            wait_all(v_v.at[sv], sem_v.at[sv])
            issue_tail(LA + g, LA, LA + NG)
            eb, l_run = probs((NP - 1) & 1, g, m, l_run)
            return o + _mm_nt(eb, v_v[sv]), l_run

        with scope("v15_loop"):
            o, l_run = lax.fori_loop(0, NG, v_step, (zero_o, zero_l))
        with scope("ffn_in"):
            acc = finish_pair(NP - 1, o, l_run, acc)
            attn = jnp.sum(acc, axis=0, keepdims=True)
            x1 = xf8 + ga * attn
            h2 = (_layernorm(x1) * (1.0 + cb) + sb).astype(jnp.bfloat16)

            wait_all(wg_v, sem_s.at[4])
            g_ = _mm(h2, wg_v[...])
        with scope("up"):
            UR = D // up_chunks
            u_ = jnp.zeros((8, F), jnp.float32)
            for i in range(up_chunks):
                wait_all(wu_v.at[pl.ds(i * UR, UR), :], sem_u.at[i])
                u_ = u_ + _mm(h2[:, i * UR:(i + 1) * UR], wu_v[i * UR:(i + 1) * UR, :])
            hh = (g_ * u_).astype(jnp.bfloat16)
        y = jnp.zeros((8, D), jnp.float32)
        for i in range(wd_chunks):
            with scope(f"wd{i}"):
                wait_all(wd_v.at[pl.ds(i * WDR, WDR), :], sem_d.at[i])
                y = y + _mm(hh[:, i * WDR:(i + 1) * WDR], wd_v[i * WDR:(i + 1) * WDR, :])
        out = x1 + gb * y
        o_ref[0] = out[0:1, :].astype(jnp.bfloat16)

    def fn(A_x, A_k_cache, A_v_cache, A_wq, A_wo, B_x, B_w_gate, B_w_up, B_w_down, c, w_mod):
        del B_x
        kt = A_k_cache.transpose(0, 1, 3, 2).reshape(HQ * DH, SK)
        vt = A_v_cache.transpose(0, 1, 3, 2).reshape(HQ * DH, SK)
        hbm = pl.BlockSpec(memory_space=pl.ANY)
        return pl.pallas_call(
            kernel,
            in_specs=[hbm] * 10,
            out_specs=pl.BlockSpec(memory_space=pltpu.VMEM),
            out_shape=jax.ShapeDtypeStruct((1, 1, D), jnp.bfloat16),
            scratch_shapes=[
                pltpu.VMEM((1, 1, D), jnp.bfloat16),
                pltpu.VMEM((1, D), jnp.bfloat16),
                pltpu.VMEM((D, 6 * D), jnp.bfloat16),
                pltpu.VMEM((D, HQ * DH), jnp.bfloat16),
                pltpu.VMEM((2, 2 * NG, PR, GC), jnp.bfloat16),
                pltpu.VMEM((HQ * DH, D), jnp.bfloat16),
                pltpu.VMEM((D, F), jnp.bfloat16),
                pltpu.VMEM((D, F), jnp.bfloat16),
                pltpu.VMEM((F, D), jnp.bfloat16),
                pltpu.VMEM((2, NG, 8, GC), jnp.float32),
                pltpu.SemaphoreType.DMA((5,)),
                pltpu.SemaphoreType.DMA((2 * NG,)),
                pltpu.SemaphoreType.DMA((2 * NG,)),
                pltpu.SemaphoreType.DMA((4,)),
                pltpu.SemaphoreType.DMA((wd_chunks,)),
                pltpu.SemaphoreType.DMA((max(up_chunks, 1),)),
            ],
            compiler_params=pltpu.CompilerParams(
                vmem_limit_bytes=100 * 1024 * 1024,
                disable_bounds_checks=None if checks else True,
                disable_semaphore_checks=not checks,
                flags=flags),
        )(A_x, c, w_mod, A_wq, kt, vt, A_wo, B_w_gate, B_w_up, B_w_down)

    return fn


@jax.jit
def pallas_adaLN_cond__sliding_block_cached__glu_gated_bilinear__decode_kernel(
    A_x, A_k_cache, A_v_cache, A_wq, A_wo, B_x, B_w_gate, B_w_up, B_w_down, c, w_mod,
):
    return _make()(A_x, A_k_cache, A_v_cache, A_wq, A_wo, B_x, B_w_gate, B_w_up, B_w_down, c, w_mod)
```

```python
import jax
import jax.numpy as jnp
from jax import lax
from jax.experimental import pallas as pl
from jax.experimental.pallas import tpu as pltpu

D = 640
HQ, DH = 32, 192
SK, W = 32768, 4096
F = 1536
EPS = 1e-5
SCORE_SCALE = DH ** -0.5 * 1.4426950408889634

PR = 2 * DH
NP = HQ // 2
GC = 512
NG = W // GC
LGNG = 3
RP = 32
LA = 7
N_PRE = 3
WQ_PRE = 20
MOD_COLS, WQ_COLS = 640, 1024
WO_ROWS = PR // NG
UP_CH, UP_ROWS = 5, D // 2 // 5
WD_CH, WD_ROWS, WD_PIECE = 6, F // 2 // 6, 32
V_PER = 2
V_SLOTS = NG // V_PER
UP_A = V_SLOTS
WD_A, WD_PER = UP_A + UP_CH, 2


def _mm(a, b):
    return jnp.dot(a, b, preferred_element_type=jnp.float32)


def _mm_nt(a, b):
    return lax.dot_general(a, b, (((1,), (1,)), ((), ())), preferred_element_type=jnp.float32)


def _layernorm(x):
    m = jnp.mean(x, axis=-1, keepdims=True)
    d = x - m
    v = jnp.mean(d * d, axis=-1, keepdims=True)
    return d * lax.rsqrt(v + EPS)


def _bf16_round(x):
    return x.astype(jnp.bfloat16).astype(jnp.float32)


def _kernel(x_hbm, c_hbm, wmod_hbm, wq_hbm, kt_hbm, vt_hbm, wo_hbm, wg_hbm, wu_hbm, wd_hbm,
            o_ref,
            x_v, c_v, wmod_v, wq_v, kv_v, wo_v, wg_v, wu_v, wd_v, s_v,
            sem_s, sem_k, sem_v, sem_o, sem_u, sem_d):
    k_v, v_v = kv_v.at[0], kv_v.at[1]
    sk = kt_hbm.shape[1]

    def kv_dma(src, dst, sem, u, g, r0, pr):
        r = pl.multiple_of(u * PR + r0, 8)
        if not isinstance(r0, int):
            r0 = pl.multiple_of(r0, 8)
        cc = pl.multiple_of(sk - W + g * GC, 128)
        slot = (u & 1) * NG + g
        pltpu.make_async_copy(src.at[pl.ds(r, RP), pl.ds(cc, GC)], dst.at[slot, pl.ds(r0, RP), :],
                              sem.at[slot]).start(priority=pr)

    def rows_dma(src, dst, sem, r, nr, pr, c0=0, nc=None, rd=None):
        nc = src.shape[1] if nc is None else nc
        r = pl.multiple_of(r, 8)
        d = dst.at[pl.ds(r, nr), pl.ds(c0, nc)] if rd is None else dst.at[pl.ds(rd, nr), :]
        pltpu.make_async_copy(src.at[pl.ds(r, nr), pl.ds(c0, nc)], d, sem).start(priority=pr)

    def wait_all(dst, sem):
        pltpu.make_async_copy(dst, dst, sem).wait()

    def halves(i):
        if isinstance(i, int):
            return i - i % 2, i % 2
        return i & ~1, i & 1

    def issue_single(src, dst, sem, u, i):
        g0, rb = halves(i)
        for j in range(2):
            for part in range(DH // 2 // RP):
                kv_dma(src, dst, sem, u, g0 + j, rb * (DH // 2) + part * RP, 0)
                kv_dma(src, dst, sem, u, g0 + j, DH + rb * (DH // 2) + part * RP, 1)

    def issue_main(t, gate):
        u = lax.shift_right_logical(t, LGNG)
        g = t & (NG - 1)
        g0, rb = halves(g)
        for j in range(2):
            for part in range(DH // RP):
                kv_dma(kt_hbm, k_v, sem_k, u + 1, g0 + j, rb * DH + part * RP, 0)
                kv_dma(vt_hbm, v_v, sem_v, u, g0 + j, rb * DH + part * RP, 1)
        rows_dma(wo_hbm, wo_v, sem_o.at[(u + 1) & 3], (u + 1) * PR + g * WO_ROWS, WO_ROWS, 0)

        def gate_rows():
            rows_dma(wg_hbm, wg_v, sem_s.at[4], t * 8, 8, 0, 0, F // 2)
            rows_dma(wg_hbm, wg_v, sem_s.at[4], t * 8, 8, 1, F // 2, F // 2)

        if gate == "while_left":
            pl.when(t < D // 8)(gate_rows)
        elif gate == "yes":
            gate_rows()

    def issue_tail(i, lo, hi):
        if lo < V_SLOTS:
            @pl.when(i < V_SLOTS)
            def _():
                for k in range(V_PER):
                    issue_single(vt_hbm, v_v, sem_v, NP - 1, i * V_PER + k)
        if lo < UP_A + UP_CH and hi > UP_A:
            @pl.when(jnp.logical_and(i >= UP_A, i < UP_A + UP_CH))
            def _():
                ch = i - UP_A
                for k in range(UP_ROWS // 8):
                    for half in range(2):
                        rows_dma(wu_hbm, wu_v.at[ch], sem_u.at[ch], half * (D // 2) + ch * UP_ROWS + k * 8, 8,
                                 half, rd=half * UP_ROWS + k * 8)
        if lo < WD_A + WD_CH // WD_PER and hi > WD_A:
            @pl.when(jnp.logical_and(i >= WD_A, i < WD_A + WD_CH // WD_PER))
            def _():
                for k in range(WD_PER):
                    ch = (i - WD_A) * WD_PER + k
                    for n in range(WD_ROWS // WD_PIECE):
                        for half in range(2):
                            rows_dma(wd_hbm, wd_v.at[ch], sem_d.at[ch],
                                     half * (F // 2) + ch * WD_ROWS + n * WD_PIECE, WD_PIECE, half,
                                     rd=half * WD_ROWS + n * WD_PIECE)

    def issue_halves(src, dst, sem, cols, lo, hi):
        rows, width = src.shape

        def body(i, _):
            for j in range(width // cols):
                for half in range(2):
                    rows_dma(src, dst, sem, half * (rows // 2) + i * 8, 8, half, j * cols, cols)

        lax.fori_loop(lo, hi, body, None)

    c_cp = pltpu.make_async_copy(c_hbm, c_v, sem_s.at[0])
    x_cp = pltpu.make_async_copy(x_hbm, x_v, sem_s.at[1])

    issue_halves(wmod_hbm, wmod_v, sem_s.at[2], MOD_COLS, 0, 2)
    c_cp.start()
    x_cp.start()
    issue_halves(wmod_hbm, wmod_v, sem_s.at[2], MOD_COLS, 2, D // 16)
    issue_halves(wq_hbm, wq_v, sem_s.at[3], WQ_COLS, 0, WQ_PRE)

    c_cp.wait()
    x_cp.wait()
    cf = c_v[...].astype(jnp.float32)
    silu_c = jnp.broadcast_to(cf * jax.nn.sigmoid(cf), (8, D)).astype(jnp.bfloat16)
    x0 = jnp.broadcast_to(x_v[0].astype(jnp.float32), (8, D))
    ln1 = _layernorm(x0)
    wait_all(wmod_v, sem_s.at[2])
    mod = _bf16_round(_mm(silu_c, wmod_v[...]))
    sa, ca, ga = mod[:, 0:D], mod[:, D:2 * D], mod[:, 2 * D:3 * D]
    sb, cb, gb = mod[:, 3 * D:4 * D], mod[:, 4 * D:5 * D], mod[:, 5 * D:6 * D]
    h1 = (ln1 * (1.0 + ca) + sa).astype(jnp.bfloat16)

    issue_halves(wq_hbm, wq_v, sem_s.at[3], WQ_COLS, WQ_PRE, D // 16)
    lax.fori_loop(0, NG, lambda i, _: issue_single(kt_hbm, k_v, sem_k, 0, i), None)
    for i in range(4):
        rows_dma(wo_hbm, wo_v, sem_o.at[0], i * (PR // 4), PR // 4, i % 2)
    lax.fori_loop(0, N_PRE, lambda t, _: issue_main(t, "yes"), None)
    wait_all(wq_v, sem_s.at[3])

    sub = lax.broadcasted_iota(jnp.int32, (8, PR), 0)
    lane = lax.broadcasted_iota(jnp.int32, (8, PR), 1)
    pair_mask = (lane >= DH).astype(jnp.int32) == sub

    def q_block(u):
        q = _mm(h1, wq_v[:, pl.ds(pl.multiple_of(u * PR, 128), PR)])
        return jnp.where(pair_mask, q, 0.0).astype(jnp.bfloat16)

    def scores(qb, par, g, m_run):
        s = _mm(qb, k_v[par * NG + g])
        s_v[par, g] = s
        for j in range(GC // 128):
            m_run = jnp.maximum(m_run, s[:, j * 128:(j + 1) * 128])
        return m_run

    def probs(par, g, m, l_run):
        e = jnp.exp2((s_v[par, g] - m) * SCORE_SCALE)
        for j in range(GC // 128):
            l_run = l_run + e[:, j * 128:(j + 1) * 128]
        return e.astype(jnp.bfloat16), l_run

    def finish_pair(u, o, l_run, acc):
        l = jnp.sum(l_run, axis=-1, keepdims=True)
        ob = jnp.where(pair_mask, o * (1.0 / l), 0.0).astype(jnp.bfloat16)
        r = pl.multiple_of(u * PR, PR)
        wait_all(wo_v.at[pl.ds(r, PR), :], sem_o.at[u & 3])
        return acc + _mm(ob, wo_v[pl.ds(r, PR), :])

    neg = jnp.full((8, 128), -jnp.inf, jnp.float32)
    zero_o = jnp.zeros((8, PR), jnp.float32)
    zero_l = jnp.zeros((8, 128), jnp.float32)

    qb0 = q_block(0)

    def k0_step(g, m_run):
        wait_all(k_v.at[g], sem_k.at[g])

        @pl.when(g < LA - N_PRE)
        def _():
            issue_main(N_PRE + g, "yes")

        return scores(qb0, 0, g, m_run)

    m = jnp.max(lax.fori_loop(0, NG, k0_step, neg), axis=-1, keepdims=True)

    def pair_body(u, carry, last):
        m, acc = carry
        qb = q_block(u + 1)
        pv = u & 1

        def step(g, c2):
            m_run, o, l_run = c2
            t = u * NG + g
            sv, skk = pv * NG + g, (1 - pv) * NG + g
            wait_all(v_v.at[sv], sem_v.at[sv])
            wait_all(k_v.at[skk], sem_k.at[skk])
            if last:
                @pl.when(g + LA < NG)
                def _():
                    issue_main(t + LA, "no")

                @pl.when(g + LA >= NG)
                def _():
                    issue_tail(g + LA - NG, 0, LA)
            else:
                issue_main(t + LA, "while_left")
            eb, l_run = probs(pv, g, m, l_run)
            o = o + _mm_nt(eb, v_v[sv])
            m_run = scores(qb, 1 - pv, g, m_run)
            return m_run, o, l_run

        m_run, o, l_run = lax.fori_loop(0, NG, step, (neg, zero_o, zero_l))
        m_new = jnp.max(m_run, axis=-1, keepdims=True)
        return m_new, finish_pair(u, o, l_run, acc)

    carry = lax.fori_loop(0, NP - 2, lambda u, cr: pair_body(u, cr, False),
                          (m, jnp.zeros((8, D), jnp.float32)))
    m, acc = pair_body(NP - 2, carry, True)

    def v_step(g, c2):
        o, l_run = c2
        sv = ((NP - 1) & 1) * NG + g
        wait_all(v_v.at[sv], sem_v.at[sv])
        issue_tail(LA + g, LA, LA + NG)
        eb, l_run = probs((NP - 1) & 1, g, m, l_run)
        return o + _mm_nt(eb, v_v[sv]), l_run

    o, l_run = lax.fori_loop(0, NG, v_step, (zero_o, zero_l))
    acc = finish_pair(NP - 1, o, l_run, acc)
    x1 = x0 + ga * jnp.sum(acc, axis=0, keepdims=True)
    h2 = (_layernorm(x1) * (1.0 + cb) + sb).astype(jnp.bfloat16)

    wait_all(wg_v, sem_s.at[4])
    gate = _mm(h2, wg_v[...])
    up = jnp.zeros((8, F), jnp.float32)
    for ch in range(UP_CH):
        wait_all(wu_v.at[ch], sem_u.at[ch])
        for half in range(2):
            r0 = half * (D // 2) + ch * UP_ROWS
            up = up + _mm(h2[:, r0:r0 + UP_ROWS], wu_v[ch, half * UP_ROWS:(half + 1) * UP_ROWS, :])
    hh = (gate * up).astype(jnp.bfloat16)
    y = jnp.zeros((8, D), jnp.float32)
    for ch in range(WD_CH):
        wait_all(wd_v.at[ch], sem_d.at[ch])
        for half in range(2):
            r0 = half * (F // 2) + ch * WD_ROWS
            y = y + _mm(hh[:, r0:r0 + WD_ROWS], wd_v[ch, half * WD_ROWS:(half + 1) * WD_ROWS, :])
    out = x1 + gb * y
    o_ref[0] = out[0:1, :].astype(jnp.bfloat16)


def _call(A_x, A_k_cache, A_v_cache, A_wq, A_wo, B_w_gate, B_w_up, B_w_down, c, w_mod,
          interpret=False, checks=False):
    sk = A_k_cache.shape[2]
    kt = A_k_cache.transpose(0, 1, 3, 2).reshape(HQ * DH, sk)
    vt = A_v_cache.transpose(0, 1, 3, 2).reshape(HQ * DH, sk)
    hbm = pl.BlockSpec(memory_space=pl.ANY)
    return pl.pallas_call(
        _kernel,
        in_specs=[hbm] * 10,
        out_specs=pl.BlockSpec(memory_space=pltpu.VMEM),
        out_shape=jax.ShapeDtypeStruct((1, 1, D), jnp.bfloat16),
        scratch_shapes=[
            pltpu.VMEM((1, 1, D), jnp.bfloat16),
            pltpu.VMEM((1, D), jnp.bfloat16),
            pltpu.VMEM((D, 6 * D), jnp.bfloat16),
            pltpu.VMEM((D, HQ * DH), jnp.bfloat16),
            pltpu.VMEM((2, 2 * NG, PR, GC), jnp.bfloat16),
            pltpu.VMEM((HQ * DH, D), jnp.bfloat16),
            pltpu.VMEM((D, F), jnp.bfloat16),
            pltpu.VMEM((UP_CH, 2 * UP_ROWS, F), jnp.bfloat16),
            pltpu.VMEM((WD_CH, 2 * WD_ROWS, D), jnp.bfloat16),
            pltpu.VMEM((2, NG, 8, GC), jnp.float32),
            pltpu.SemaphoreType.DMA((5,)),
            pltpu.SemaphoreType.DMA((2 * NG,)),
            pltpu.SemaphoreType.DMA((2 * NG,)),
            pltpu.SemaphoreType.DMA((4,)),
            pltpu.SemaphoreType.DMA((UP_CH,)),
            pltpu.SemaphoreType.DMA((WD_CH,)),
        ],
        interpret=interpret,
        compiler_params=pltpu.CompilerParams(
            vmem_limit_bytes=100 * 1024 * 1024,
            disable_bounds_checks=not checks,
            disable_semaphore_checks=not checks),
    )(A_x, c, w_mod, A_wq, kt, vt, A_wo, B_w_gate, B_w_up, B_w_down)


@jax.jit
def pallas_adaLN_cond__sliding_block_cached__glu_gated_bilinear__decode_kernel(
    A_x: jax.Array,
    A_k_cache: jax.Array,
    A_v_cache: jax.Array,
    A_wq: jax.Array,
    A_wo: jax.Array,
    B_x: jax.Array,
    B_w_gate: jax.Array,
    B_w_up: jax.Array,
    B_w_down: jax.Array,
    c: jax.Array,
    w_mod: jax.Array,
):
    del B_x
    return _call(A_x, A_k_cache, A_v_cache, A_wq, A_wo, B_w_gate, B_w_up, B_w_down, c, w_mod)
```
